```python
import jax
import jax.numpy as jnp

def _softmax(x, axis=-1):
    return jax.nn.softmax(x, axis=axis)
def _gelu(x):
    return jax.nn.gelu(x, approximate=True)
def _silu(x):
    return jax.nn.silu(x)
def _sigmoid(x):
    return jax.nn.sigmoid(x)
def _layernorm(x, axis=-1, eps=1e-5):
    m = jnp.mean(x, axis=axis, keepdims=True)
    v = jnp.var(x, axis=axis, keepdims=True)
    return (x - m) / jnp.sqrt(v + eps)
def _scatter_add(tgt, idx, src, axis=0):
    return tgt.at[idx].add(src)
def _segment_sum(src, seg, n):
    return jax.ops.segment_sum(src, seg, n)
class _Rng:
    def __init__(self, key):
        self._k = key
    def _next(self):
        self._k, sub = jax.random.split(self._k)
        return sub
    def normal(self, shape):
        return jax.random.normal(self._next(), shape, dtype=jnp.bfloat16)
    def randint(self, lo, hi, shape):
        return jax.random.randint(self._next(), shape, lo, hi, dtype=jnp.int32)
    def uniform(self, shape, lo=0.0, hi=1.0):
        return jax.random.uniform(self._next(), shape, jnp.bfloat16, lo, hi)
    def permutation(self, n):
        return jax.random.permutation(self._next(), n)


kernel_name = 'standalone__fft_conv__vision'

def setup_inputs():
    _rng = _Rng(jax.random.key(int.from_bytes(__import__("os").urandom(4), "little")))
    _w = (lambda a: (lambda t: t.astype(jnp.bfloat16) if jnp.issubdtype(t.dtype, jnp.floating) else t)(jnp.asarray(a)))
    H = W = 224
    C = 96
    K = 7
    return {
        "x": _w((lambda *s: _rng.normal(s) * 0.05)(1, H, W, C)),
        "w": _w((lambda *s: _rng.normal(s) * 0.05)(K, K, C, C)),
    }

def reference(x, w):
    B, H, W, C = x.shape
    K = w.shape[0]
    wp = jnp.pad(w, ((0, H - K), (0, W - K), (0, 0), (0, 0)))
    Xf = (lambda x, axes=(-2,-1): jnp.fft.rfft2(x.astype(jnp.float32), axes=axes))(x, axes=(1, 2))
    Wf = (lambda x, axes=(-2,-1): jnp.fft.rfft2(x.astype(jnp.float32), axes=axes))(wp, axes=(0, 1))
    Yf = jnp.einsum('bhwi,hwio->bhwo', Xf, Wf)
    y = (lambda x, s, axes=(-2,-1): jnp.fft.irfft2(x, s=s, axes=axes).astype(jnp.bfloat16))(Yf, (H, W), axes=(1, 2))
    return y
```

```python
import math

import numpy as np
import jax
import jax.numpy as jnp
from jax import lax
import jax.experimental.pallas as pl
import jax.experimental.pallas.tpu as pltpu

H = 224
W = 224
C = 96
K = 7
T = 20
V = 14
NT = 16
NSLOT = H + 6
NPL = 600
KW = 56


def _plane_fwd(p, b):
    if p == 0:
        return 1.0
    if p == T - 1:
        return -1.0 if b % 2 else 1.0
    v = (p + 1) // 2
    ang = 2.0 * math.pi * v * b / T
    return math.cos(ang) if p % 2 == 1 else -math.sin(ang)


def _plane_inv(p, b):
    if p == 0:
        return 1.0
    if p == T - 1:
        return -1.0 if b % 2 else 1.0
    v = (p + 1) // 2
    ang = 2.0 * math.pi * v * b / T
    return 2.0 * math.cos(ang) if p % 2 == 1 else -2.0 * math.sin(ang)


def _make_f():
    f = np.zeros((2, 8 * T, 128), np.float32)
    for g in range(2):
        for tl in range(8):
            for b in range(T):
                w = V * (8 * g + tl) - 6 + b
                if g == 0:
                    lane = w if w >= 0 else 112 + (w + 6)
                else:
                    lane = w if w < 128 else w - 128
                for p in range(T):
                    f[g, tl * T + p, lane] = _plane_fwd(p, b)
    return f


def _make_g():
    g = np.zeros((4 * V, 4 * T), np.float32)
    for tl in range(4):
        for b in range(6, T):
            for p in range(T):
                g[tl * V + b - 6, tl * T + p] = _plane_inv(p, b)
    return g


def _freq_list():
    out = []
    q = 0
    for v in range(1, 10):
        for u in range(T):
            out.append((u, v, q, False))
            q += 3
    for v in (0, 10):
        for u in range(11):
            real = u in (0, 10)
            out.append((u, v, q, real))
            q += 1 if real else 3
    assert q == 598
    return out


def _make_c():
    c = np.zeros((NPL, KW), np.float64)
    for (u, v, q, real) in _freq_list():
        for a in range(K):
            for b in range(K):
                ang = -2.0 * math.pi * (u * a + v * b) / T
                wr = math.cos(ang) / (T * T)
                wi = math.sin(ang) / (T * T)
                if real:
                    c[q, a * K + b] = wr
                else:
                    c[q, a * K + b] = wr
                    c[q + 1, a * K + b] = wr + wi
                    c[q + 2, a * K + b] = wi - wr
    return c.astype(np.float32)


_F = _make_f()
_G = _make_g()
_CW = _make_c()


def _neg(a):
    return None if a is None else (a[0], -a[1])


def _add(a, b):
    if a is None:
        return b
    if b is None:
        return a
    if a[1] == b[1]:
        return (a[0] + b[0], a[1])
    if a[1] > 0:
        return (a[0] - b[0], 1)
    return (b[0] - a[0], 1)


def _sub(a, b):
    return _add(a, _neg(b))


def _mul(c, a):
    if a is None:
        return None
    return (a[0] * np.float32(c * a[1]), 1)


def _cadd(a, b):
    return (_add(a[0], b[0]), _add(a[1], b[1]))


def _csub(a, b):
    return (_sub(a[0], b[0]), _sub(a[1], b[1]))


def _cscale(c, a):
    return (_mul(c, a[0]), _mul(c, a[1]))


def _dft4(x):
    s0, d0 = _cadd(x[0], x[2]), _csub(x[0], x[2])
    s1, d1 = _cadd(x[1], x[3]), _csub(x[1], x[3])
    x1 = (_add(d0[0], d1[1]), _sub(d0[1], d1[0]))
    x3 = (_sub(d0[0], d1[1]), _add(d0[1], d1[0]))
    return [_cadd(s0, s1), x1, _csub(s0, s1), x3]


_C1 = math.cos(2 * math.pi / 5)
_C2 = math.cos(4 * math.pi / 5)
_S1 = math.sin(2 * math.pi / 5)
_S2 = math.sin(4 * math.pi / 5)


def _dft5(x):
    t1, t3 = _cadd(x[1], x[4]), _csub(x[1], x[4])
    t2, t4 = _cadd(x[2], x[3]), _csub(x[2], x[3])
    t5 = _cadd(t1, t2)
    x0 = _cadd(x[0], t5)
    m2 = _cadd(x[0], _cscale((_C1 + _C2) / 2, t5))
    m3 = _cscale((_C1 - _C2) / 2, _csub(t1, t2))
    s1, s2 = _cadd(m2, m3), _csub(m2, m3)
    u = _cadd(_cscale(_S1, t3), _cscale(_S2, t4))
    v = _csub(_cscale(_S2, t3), _cscale(_S1, t4))
    x1 = (_add(s1[0], u[1]), _sub(s1[1], u[0]))
    x4 = (_sub(s1[0], u[1]), _add(s1[1], u[0]))
    x2 = (_add(s2[0], v[1]), _sub(s2[1], v[0]))
    x3 = (_sub(s2[0], v[1]), _add(s2[1], v[0]))
    return [x0, x1, x2, x3, x4]


def _fft20(x, real_input=False):
    a = [_dft4([x[(5 * n1 + 4 * n2) % 20] for n1 in range(4)]) for n2 in range(5)]
    out = [None] * 20
    for k1 in range(4):
        if real_input and k1 == 3:
            continue
        r = _dft5([a[n2][k1] for n2 in range(5)])
        for k2 in range(5):
            out[(5 * k1 + 16 * k2) % 20] = r[k2]
            if real_input and k1 == 1:
                out[(-(5 * k1 + 16 * k2)) % 20] = (r[k2][0], _neg(r[k2][1]))
    return out


def _ifft20(y):
    r = _fft20([(b, a) for (a, b) in y])
    return [(b, a) for (a, b) in r]


def _val(a):
    if a[1] > 0:
        return a[0]
    return -a[0]


def _pos(arr):
    return (arr, 1)


NCH = 8
HC = H // NCH


def _kernel(x_hbm, w_ref, f_ref, g_ref, c_ref, o_hbm,
            xbuf, obuf, xy1, wf, what, x2, y2, isem, osem):
    f32 = jnp.float32

    def in_copy(k):
        return pltpu.make_async_copy(
            x_hbm.at[pl.ds(k * HC, HC)], xbuf.at[pl.ds(k * HC, HC)], isem.at[k])

    def out_copy(k):
        return pltpu.make_async_copy(
            obuf.at[pl.ds(k * HC, HC)], o_hbm.at[pl.ds(k * HC, HC)], osem.at[k])

    for k in range(NCH):
        in_copy(k).start()

    wf[pl.ds(0, K * K * C), :] = w_ref[...].astype(f32)
    wf[pl.ds(K * K * C, (KW - K * K) * C), :] = jnp.zeros(((KW - K * K) * C, C), f32)

    def w_body(i, carry):
        rhs = wf[pl.ds(i, KW, stride=C), :]
        what[pl.ds(i, NPL, stride=C), :] = jnp.dot(
            c_ref[...], rhs, preferred_element_type=f32)
        return carry

    lax.fori_loop(0, C, w_body, 0)

    def s1_row(h):
        xa = x_ref_row(h, 0, 128)
        xb = x_ref_row(h, 128, 96)
        w0 = jnp.concatenate([xa[:, :112], xb[:, 90:96], xa[:, 118:128]], axis=1)
        w1 = jnp.concatenate([xb, xa[:, 96:128]], axis=1)
        nt = (((1,), (1,)), ((), ()))
        r0 = lax.dot_general(f_ref[0], w0, nt, preferred_element_type=f32)
        r1 = lax.dot_general(f_ref[1], w1, nt, preferred_element_type=f32)
        xy1[h + 6, pl.ds(0, 160), :] = r0
        xy1[h + 6, pl.ds(160, 160), :] = r1

        @pl.when(h >= H - 6)
        def _():
            hh = jnp.maximum(h - (H - 6), 0)
            xy1[hh, pl.ds(0, 160), :] = r0
            xy1[hh, pl.ds(160, 160), :] = r1

    def x_ref_row(h, lo, n):
        return xbuf[h, :, pl.ds(lo, n)]

    for k in range(NCH):
        in_copy(k).wait()

        def s1_body(j, carry, k=k):
            s1_row(k * HC + j)
            return carry

        lax.fori_loop(0, HC, s1_body, 0)

    def ld1(slot, g, p):
        return xy1[slot, pl.ds(g * 160 + p, 8, stride=T), :]

    def st1(slot, g, p, val):
        xy1[slot, pl.ds(g * 160 + p, 8, stride=T), :] = val

    def st_planes(q, row, z, real):
        if real:
            x2[q, pl.ds(row, 8), :] = _val(z[0])
        else:
            zr, zi = _val(z[0]), _val(z[1])
            x2[q, pl.ds(row, 8), :] = zr + zi
            x2[q + 1, pl.ds(row, 8), :] = zi
            x2[q + 2, pl.ds(row, 8), :] = zr

    def s3(q, wq, u_slot, real):
        def mm(j):
            return jnp.dot(x2[q + j], what[pl.ds((wq + j) * C, C), :],
                           preferred_element_type=f32)
        if real:
            y2[2 * u_slot] = mm(0)
        else:
            k1, k2, k3 = mm(0), mm(1), mm(2)
            y2[2 * u_slot] = k1 - k2
            y2[2 * u_slot + 1] = k1 + k3

    def complex_step(v, carry):
        p_re, p_im = 2 * v - 1, 2 * v

        def s2_body(th, c2):
            for g in range(2):
                z = [(_pos(ld1(V * th + a, g, p_re)), _pos(ld1(V * th + a, g, p_im)))
                     for a in range(T)]
                zf = _fft20(z)
                row = pl.multiple_of(th * 16 + g * 8, 8)
                for u in range(T):
                    st_planes(3 * u, row, zf[u], False)
            return c2

        lax.fori_loop(0, NT, s2_body, 0)

        def s3_body(u, c2):
            s3(3 * u, 60 * (v - 1) + 3 * u, u, False)
            return c2

        lax.fori_loop(0, T, s3_body, 0)

        def s4_body(th, c2):
            for g in range(2):
                row = pl.multiple_of(th * 16 + g * 8, 8)
                z = [(_pos(y2[2 * u, pl.ds(row, 8), :]), _pos(y2[2 * u + 1, pl.ds(row, 8), :]))
                     for u in range(T)]
                r = _ifft20(z)
                for a in range(6, T):
                    st1(V * th + a, g, p_re, _val(r[a][0]))
                    st1(V * th + a, g, p_im, _val(r[a][1]))
            return c2

        lax.fori_loop(0, NT, s4_body, 0)
        return carry

    lax.fori_loop(1, 10, complex_step, 0)

    def real_q(u):
        return 0 if u == 0 else (28 if u == 10 else 1 + 3 * (u - 1))

    for vi, p in enumerate((0, T - 1)):
        def s2r_body(th, c2, p=p):
            for g in range(2):
                z = [(_pos(ld1(V * th + a, g, p)), None) for a in range(T)]
                zf = _fft20(z, real_input=True)
                row = pl.multiple_of(th * 16 + g * 8, 8)
                for u in range(11):
                    st_planes(real_q(u), row, zf[u], u in (0, 10))
            return c2

        lax.fori_loop(0, NT, s2r_body, 0)

        for u in range(11):
            s3(real_q(u), 540 + 29 * vi + real_q(u), u, u in (0, 10))

        def s4r_body(th, c2, p=p):
            for g in range(2):
                row = pl.multiple_of(th * 16 + g * 8, 8)
                z = [None] * T
                for u in range(11):
                    re = _pos(y2[2 * u, pl.ds(row, 8), :])
                    im = None if u in (0, 10) else _pos(y2[2 * u + 1, pl.ds(row, 8), :])
                    z[u] = (re, im)
                    if 0 < u < 10:
                        z[T - u] = (re, _neg(im))
                r = _ifft20(z)
                for a in range(6, T):
                    st1(V * th + a, g, p, _val(r[a][0]))
            return c2

        lax.fori_loop(0, NT, s4r_body, 0)

    for k in range(NCH):
        def s5_body(j, carry, k=k):
            h = k * HC + j
            parts = [jnp.dot(g_ref[...], xy1[h + 6, pl.ds(80 * jj, 80), :],
                             preferred_element_type=f32) for jj in range(4)]
            y = jnp.concatenate(parts, axis=0)
            obuf[h] = y.T.astype(jnp.bfloat16)
            return carry

        lax.fori_loop(0, HC, s5_body, 0)
        out_copy(k).start()

    for k in range(NCH):
        out_copy(k).wait()


@jax.jit
def pallas_standalone__fft_conv__vision_kernel(x: jax.Array, w: jax.Array):
    assert x.shape == (1, H, W, C) and w.shape == (K, K, C, C)
    xt = jnp.transpose(x.reshape(H, W, C), (0, 2, 1))
    w2 = w.reshape(K * K * C, C)
    vmem = pl.BlockSpec(memory_space=pltpu.VMEM)
    out = pl.pallas_call(
        _kernel,
        out_shape=jax.ShapeDtypeStruct((H, C, W), jnp.bfloat16),
        in_specs=[pl.BlockSpec(memory_space=pl.ANY), vmem, vmem, vmem, vmem],
        out_specs=pl.BlockSpec(memory_space=pl.ANY),
        scratch_shapes=[
            pltpu.VMEM((H, C, W), jnp.bfloat16),
            pltpu.VMEM((H, C, W), jnp.bfloat16),
            pltpu.VMEM((NSLOT, 2 * 8 * T, C), jnp.float32),
            pltpu.VMEM((KW * C, C), jnp.float32),
            pltpu.VMEM((NPL * C, C), jnp.float32),
            pltpu.VMEM((60, 256, C), jnp.float32),
            pltpu.VMEM((40, 256, C), jnp.float32),
            pltpu.SemaphoreType.DMA((NCH,)),
            pltpu.SemaphoreType.DMA((NCH,)),
        ],
        compiler_params=pltpu.CompilerParams(vmem_limit_bytes=126 * 1024 * 1024),
        name="fft_conv_vision",
    )(xt, w2, _F.astype(jnp.bfloat16), _G, _CW)
    return jnp.transpose(out, (0, 2, 1)).reshape(1, H, W, C)
```

```python
import math

import numpy as np
import jax
import jax.numpy as jnp
from jax import lax
import jax.experimental.pallas as pl
import jax.experimental.pallas.tpu as pltpu

H = 224
W = 224
C = 96
K = 7
T = 20
V = 14
NT = 16
NSLOT = H + 6
NPL = 598
SH = 3

_FLAGS = {}
F32 = jnp.float32
BF16 = jnp.bfloat16


def _plane_fwd(p, b):
    if p == 0:
        return 1.0
    if p == T - 1:
        return -1.0 if b % 2 else 1.0
    v = (p + 1) // 2
    ang = 2.0 * math.pi * v * b / T
    return math.cos(ang) if p % 2 == 1 else -math.sin(ang)


def _plane_inv(p, b):
    if p == 0:
        return 1.0
    if p == T - 1:
        return -1.0 if b % 2 else 1.0
    v = (p + 1) // 2
    ang = 2.0 * math.pi * v * b / T
    return 2.0 * math.cos(ang) if p % 2 == 1 else -2.0 * math.sin(ang)


def _vp(v, pl_):
    if v == 0:
        return 0 if pl_ == 0 else T - 1
    return 2 * v - 1 + pl_


def _make_f():
    f = np.zeros((2, 8 * T, 128), np.float32)
    for g in range(2):
        for tl in range(8):
            for b in range(T):
                w = V * (8 * g + tl) - 6 + b
                if g == 0:
                    lane = w if w >= 0 else 112 + (w + 6)
                else:
                    lane = w if w < 128 else w - 128
                for v in range(10):
                    for pl_ in range(2):
                        f[g, v * 16 + tl * 2 + pl_, lane] = _plane_fwd(_vp(v, pl_), b)
    return f


def _make_g():
    g = np.zeros((4 * V, 4 * T), np.float32)
    for tl in range(4):
        for b in range(V):
            for v in range(10):
                for pl_ in range(2):
                    g[tl * V + b, v * 8 + tl * 2 + pl_] = _plane_inv(_vp(v, pl_), b + SH)
    return g


_F = _make_f()
_G = _make_g()


def _real_q(u):
    return 0 if u == 0 else (28 if u == 10 else 1 + 3 * (u - 1))


def _neg(a):
    return None if a is None else (a[0], -a[1])


def _add(a, b):
    if a is None:
        return b
    if b is None:
        return a
    if a[1] == b[1]:
        return (a[0] + b[0], a[1])
    if a[1] > 0:
        return (a[0] - b[0], 1)
    return (b[0] - a[0], 1)


def _sub(a, b):
    return _add(a, _neg(b))


def _mul(c, a):
    if a is None or abs(c) < 1e-12:
        return None
    if abs(abs(c) - 1.0) < 1e-12:
        return (a[0], a[1] * (1 if c > 0 else -1))
    return (a[0] * np.float32(c * a[1]), 1)


def _cadd(a, b):
    return (_add(a[0], b[0]), _add(a[1], b[1]))


def _csub(a, b):
    return (_sub(a[0], b[0]), _sub(a[1], b[1]))


def _cscale(c, a):
    return (_mul(c, a[0]), _mul(c, a[1]))


def _dft4(x):
    s0, d0 = _cadd(x[0], x[2]), _csub(x[0], x[2])
    s1, d1 = _cadd(x[1], x[3]), _csub(x[1], x[3])
    x1 = (_add(d0[0], d1[1]), _sub(d0[1], d1[0]))
    x3 = (_sub(d0[0], d1[1]), _add(d0[1], d1[0]))
    return [_cadd(s0, s1), x1, _csub(s0, s1), x3]


_C1 = math.cos(2 * math.pi / 5)
_C2 = math.cos(4 * math.pi / 5)
_S1 = math.sin(2 * math.pi / 5)
_S2 = math.sin(4 * math.pi / 5)


def _dft5(x):
    t1, t3 = _cadd(x[1], x[4]), _csub(x[1], x[4])
    t2, t4 = _cadd(x[2], x[3]), _csub(x[2], x[3])
    t5 = _cadd(t1, t2)
    x0 = _cadd(x[0], t5)
    m2 = _cadd(x[0], _cscale((_C1 + _C2) / 2, t5))
    m3 = _cscale((_C1 - _C2) / 2, _csub(t1, t2))
    s1, s2 = _cadd(m2, m3), _csub(m2, m3)
    u = _cadd(_cscale(_S1, t3), _cscale(_S2, t4))
    v = _csub(_cscale(_S2, t3), _cscale(_S1, t4))
    x1 = (_add(s1[0], u[1]), _sub(s1[1], u[0]))
    x4 = (_sub(s1[0], u[1]), _add(s1[1], u[0]))
    x2 = (_add(s2[0], v[1]), _sub(s2[1], v[0]))
    x3 = (_sub(s2[0], v[1]), _add(s2[1], v[0]))
    return [x0, x1, x2, x3, x4]


def _fft20(load, emit, inverse=False, real_input=False):
    def sw(z):
        return (z[1], z[0]) if inverse else z

    a = [_dft4([sw(load((5 * n1 + 4 * n2) % 20)) for n1 in range(4)]) for n2 in range(5)]
    for k1 in range(4):
        if real_input and k1 == 3:
            continue
        r = _dft5([a[n2][k1] for n2 in range(5)])
        for k2 in range(5):
            k = (5 * k1 + 16 * k2) % 20
            emit(k, sw(r[k2]))
            if real_input and k1 == 1:
                emit(20 - k, (r[k2][0], _neg(r[k2][1])))


def _val(a):
    return a[0] if a[1] > 0 else -a[0]


def _pos(arr):
    return (arr, 1)


def _sym7(x, scale=1.0):
    sm = [_add(x[3 + j], x[3 - j]) for j in (1, 2, 3)]
    df = [_sub(x[3 + j], x[3 - j]) for j in (1, 2, 3)]
    x0 = _mul(scale, x[3])

    def cs(k):
        acc = x0
        for j in (1, 2, 3):
            acc = _add(acc, _mul(scale * math.cos(2 * math.pi * k * j / T), sm[j - 1]))
        return acc

    def sn(k):
        acc = None
        for j in (1, 2, 3):
            acc = _add(acc, _mul(scale * math.sin(2 * math.pi * k * j / T), df[j - 1]))
        return acc

    return cs, sn


NCH = 8
HC = H // NCH
NQ = 4


def _kernel(x_hbm, w_ref, f_ref, g_ref, o_hbm,
            xbuf, obuf, wf, wt, what, x2a, x2b, y2a, y2b, isem, osem, *xy):
    x2 = (x2a, x2b)
    y2 = (y2a, y2b)

    def in_copy(k):
        return pltpu.make_async_copy(
            x_hbm.at[pl.ds(k * HC, HC)], xbuf.at[pl.ds(k * HC, HC)], isem.at[k])

    def out_copy(k):
        return pltpu.make_async_copy(
            obuf.at[pl.ds(k * HC, HC)], o_hbm.at[pl.ds(k * HC, HC)], osem.at[k])

    for k in range(NCH):
        in_copy(k).start()

    wf[...] = w_ref[...].astype(F32)

    def w_block(ib):
        rows = pl.ds(pl.multiple_of(ib * 8, 8), 8)
        for a in range(K):
            cs, sn = _sym7([_pos(wf[a * K + b, rows, :]) for b in range(K)], 1.0 / T)
            for v in range(11):
                wt[a, 2 * v if v < 10 else 1] = _val(cs(v))
                if 0 < v < 10:
                    wt[a, 2 * v + 1] = _val(_neg(sn(v)))

        def put(q, wr, wi):
            what[q, rows, :] = _val(wr)
            if wi is not None:
                what[q + 1, rows, :] = _val(_add(wr, wi))
                what[q + 2, rows, :] = _val(_sub(wi, wr))

        for v in range(11):
            rc, rs = _sym7([_pos(wt[a, 2 * v if v < 10 else 1]) for a in range(K)], 1.0 / T)
            if v in (0, 10):
                base = 540 + (0 if v == 0 else 29)
                for u in range(11):
                    if u in (0, 10):
                        put(base + _real_q(u), rc(u), None)
                    else:
                        put(base + _real_q(u), rc(u), _neg(rs(u)))
                continue
            ic, is_ = _sym7([_pos(wt[a, 2 * v + 1]) for a in range(K)], 1.0 / T)
            base = 60 * (v - 1)
            for u in range(11):
                a_, b_ = rc(u), ic(u)
                if u in (0, 10):
                    put(base + 3 * u, a_, b_)
                else:
                    c_, d_ = rs(u), is_(u)
                    put(base + 3 * u, _add(a_, d_), _sub(b_, c_))
                    put(base + 3 * (T - u), _sub(a_, d_), _add(b_, c_))

    def w_body(ib, carry):
        w_block(ib)
        return carry

    lax.fori_loop(0, C // 8, w_body, 0)

    nt = (((1,), (1,)), ((), ()))

    def s1_row(h):
        xa = xbuf[h, :, pl.ds(0, 128)]
        xb = xbuf[h, :, pl.ds(128, 96)]
        w0 = jnp.concatenate([xa[:, :112], xb[:, 90:96], xa[:, 118:128]], axis=1)
        w1 = jnp.concatenate([xb, xa[:, 96:128]], axis=1)
        r0 = lax.dot_general(f_ref[0], w0, nt, preferred_element_type=F32)
        r1 = lax.dot_general(f_ref[1], w1, nt, preferred_element_type=F32)
        return r0, r1

    def s1_body(k, carry):
        in_copy(k).wait()
        for j in range(HC):
            h = k * HC + j
            r0, r1 = s1_row(h)
            for v in range(10):
                xy[v][h + 6, pl.ds(0, 16), :] = r0[16 * v:16 * v + 16]
                xy[v][h + 6, pl.ds(16, 16), :] = r1[16 * v:16 * v + 16]
        return carry

    lax.fori_loop(0, NCH, s1_body, 0)
    for v in range(10):
        xy[v][pl.ds(0, 6)] = xy[v][pl.ds(H, 6)]

    def ld1(slot, g, v, part):
        return xy[v][slot, pl.ds(g * 16 + part, 8, stride=2), :]

    def st1(slot, g, v, part, val):
        xy[v][slot, pl.ds(g * 16 + part, 8, stride=2), :] = val

    def s2_one(kind, v, par, th, g):
        row = pl.ds(pl.multiple_of(th * 16 + g * 8, 8), 8)

        def put(q, z):
            if z[1] is None:
                x2[par][q, row, :] = _val(z[0])
            else:
                x2[par][q, row, :] = _val(_add(z[0], z[1]))
                x2[par][q + 1, row, :] = _val(z[1])
                x2[par][q + 2, row, :] = _val(z[0])

        if kind == "c":
            _fft20(lambda a: (_pos(ld1(V * th + a, g, v, 0)), _pos(ld1(V * th + a, g, v, 1))),
                   lambda u, z: put(3 * u, z))
        else:
            for vi in range(2):
                def emit(u, z, vi=vi):
                    if u <= 10:
                        put(29 * vi + _real_q(u), (z[0], None) if u in (0, 10) else z)
                _fft20(lambda a, vi=vi: (_pos(ld1(V * th + a, g, 0, vi)), None), emit,
                       real_input=True)

    def s3_freq(par, q, wq, slot, real):
        def mm(j):
            return jnp.dot(x2[par][q + j], what[wq + j], preferred_element_type=F32)
        if real:
            y2[par][2 * slot] = mm(0)
        else:
            k1, k2, k3 = mm(0), mm(1), mm(2)
            y2[par][2 * slot] = k1 - k2
            y2[par][2 * slot + 1] = k1 + k3

    def s3_piece(kind, v, par, t):
        if kind == "c":
            return [lambda i=i: s3_freq(par, 3 * (5 * t + i), 60 * (v - 1) + 3 * (5 * t + i),
                                        5 * t + i, False) for i in range(5)]
        freqs = [(vi, u) for vi in range(2) for u in range(11)]
        mine = freqs[t::NQ]
        return [lambda vi=vi, u=u: s3_freq(par, 29 * vi + _real_q(u),
                                           540 + 29 * vi + _real_q(u), 11 * vi + u, u in (0, 10))
                for (vi, u) in mine]

    def s4_one(kind, v, par, th, g):
        row = pl.ds(pl.multiple_of(th * 16 + g * 8, 8), 8)
        if kind == "c":
            def emit(a, z):
                if SH <= a < SH + V:
                    st1(V * th + a - SH + 6, g, v, 0, _val(z[0]))
                    st1(V * th + a - SH + 6, g, v, 1, _val(z[1]))
            _fft20(lambda u: (_pos(y2[par][2 * u, row, :]), _pos(y2[par][2 * u + 1, row, :])),
                   emit, inverse=True)
        else:
            for vi in range(2):
                cache = {}

                def load(u, vi=vi, cache=cache):
                    uu = u if u <= 10 else T - u
                    if uu not in cache:
                        re = _pos(y2[par][2 * (11 * vi + uu), row, :])
                        im = None if uu in (0, 10) else _pos(y2[par][2 * (11 * vi + uu) + 1, row, :])
                        cache[uu] = (re, im)
                    re, im = cache[uu]
                    return (re, im) if u <= 10 else (re, _neg(im))

                def emit(a, z, vi=vi):
                    if SH <= a < SH + V:
                        st1(V * th + a - SH + 6, g, 0, vi, _val(z[0]))
                _fft20(load, emit, inverse=True)

    def slot(s2, s3, s4):
        def piece(t):
            mm = s3_piece(s3[0], s3[1], s3[2], t) if s3 else []
            n = 2 * NT // NQ
            for i in range(n):
                th, g = t * (NT // NQ) + i // 2, i % 2
                lo, hi = i * len(mm) // n, (i + 1) * len(mm) // n
                for f in mm[lo:hi]:
                    f()
                if s2:
                    s2_one(s2[0], s2[1], s2[2], th, g)
                if s4:
                    s4_one(s4[0], s4[1], s4[2], th, g)

        if s3 and s3[0] == "r":
            for t in range(NQ):
                piece(t)
        else:
            def body(t, carry):
                piece(t)
                return carry
            lax.fori_loop(0, NQ, body, 0)

    slot(("c", 1, 0), None, None)
    slot(("c", 2, 1), ("c", 1, 0), None)
    for v in range(3, 10):
        par = v % 2
        slot(("c", v, 1 - par), ("c", v - 1, par), ("c", v - 2, 1 - par))
    slot(("r", 0, 1), ("c", 9, 0), ("c", 8, 1))
    slot(None, ("r", 0, 1), ("c", 9, 0))
    slot(None, None, ("r", 0, 1))

    def s5_body(k, carry):
        for j in range(HC):
            h = k * HC + j
            parts = [jnp.dot(g_ref[...],
                             jnp.concatenate([xy[v][h + 6, pl.ds(8 * jj, 8), :]
                                              for v in range(10)], axis=0),
                             preferred_element_type=F32) for jj in range(4)]
            y = jnp.concatenate(parts, axis=0)
            obuf[h] = y.T.astype(BF16)
        out_copy(k).start()
        return carry

    lax.fori_loop(0, NCH, s5_body, 0)
    for k in range(NCH):
        out_copy(k).wait()


@jax.jit
def pallas_standalone__fft_conv__vision_kernel(x: jax.Array, w: jax.Array):
    assert x.shape == (1, H, W, C) and w.shape == (K, K, C, C)
    xt = jnp.transpose(x.reshape(H, W, C), (0, 2, 1))
    w2 = w.reshape(K * K, C, C)
    vmem = pl.BlockSpec(memory_space=pltpu.VMEM)
    out = pl.pallas_call(
        _kernel,
        out_shape=jax.ShapeDtypeStruct((H, C, W), BF16),
        in_specs=[pl.BlockSpec(memory_space=pl.ANY), vmem, vmem, vmem],
        out_specs=pl.BlockSpec(memory_space=pl.ANY),
        scratch_shapes=[
            pltpu.VMEM((H, C, W), BF16),
            pltpu.VMEM((H, C, W), BF16),
            pltpu.VMEM((K * K, C, C), F32),
            pltpu.VMEM((K, T, 8, C), F32),
            pltpu.VMEM((NPL, C, C), F32),
            pltpu.VMEM((60, 256, C), F32),
            pltpu.VMEM((60, 256, C), F32),
            pltpu.VMEM((44, 256, C), F32),
            pltpu.VMEM((44, 256, C), F32),
            pltpu.SemaphoreType.DMA((NCH,)),
            pltpu.SemaphoreType.DMA((NCH,)),
        ] + [pltpu.VMEM((NSLOT, 32, C), F32) for _ in range(10)],
        compiler_params=pltpu.CompilerParams(vmem_limit_bytes=127 * 1024 * 1024, flags=_FLAGS),
        name="fft_conv_vision",
    )(xt, w2, _F.astype(BF16), _G)
    return jnp.transpose(out, (0, 2, 1)).reshape(1, H, W, C)
```

```python
import math

import numpy as np
import jax
import jax.numpy as jnp
from jax import lax
import jax.experimental.pallas as pl
import jax.experimental.pallas.tpu as pltpu

H = 224
W = 224
C = 96
K = 7
T = 20
V = 14
NT = 16
NSLOT = H + 6
NPL = 598
SH = 3

_FLAGS = {}
F32 = jnp.float32
BF16 = jnp.bfloat16


def _plane_fwd(p, b):
    if p == 0:
        return 1.0
    if p == T - 1:
        return -1.0 if b % 2 else 1.0
    v = (p + 1) // 2
    ang = 2.0 * math.pi * v * b / T
    return math.cos(ang) if p % 2 == 1 else -math.sin(ang)


def _plane_inv(p, b):
    if p == 0:
        return 1.0
    if p == T - 1:
        return -1.0 if b % 2 else 1.0
    v = (p + 1) // 2
    ang = 2.0 * math.pi * v * b / T
    return 2.0 * math.cos(ang) if p % 2 == 1 else -2.0 * math.sin(ang)


def _vp(v, pl_):
    if v == 0:
        return 0 if pl_ == 0 else T - 1
    return 2 * v - 1 + pl_


def _make_f():
    f = np.zeros((2, 8 * T, 128), np.float32)
    for g in range(2):
        for tl in range(8):
            for b in range(T):
                w = V * (8 * g + tl) - 6 + b
                if g == 0:
                    lane = w if w >= 0 else 112 + (w + 6)
                else:
                    lane = w if w < 128 else w - 128
                for v in range(10):
                    for pl_ in range(2):
                        f[g, v * 16 + tl * 2 + pl_, lane] = _plane_fwd(_vp(v, pl_), b)
    return f


def _make_g():
    g = np.zeros((4 * V, 4 * T), np.float32)
    for tl in range(4):
        for b in range(V):
            for v in range(10):
                for pl_ in range(2):
                    g[tl * V + b, v * 8 + tl * 2 + pl_] = _plane_inv(_vp(v, pl_), b + SH)
    return g


_F = _make_f()
_G = _make_g()


def _real_q(u):
    return 0 if u == 0 else (28 if u == 10 else 1 + 3 * (u - 1))


def _neg(a):
    return None if a is None else (a[0], -a[1])


def _add(a, b):
    if a is None:
        return b
    if b is None:
        return a
    if a[1] == b[1]:
        return (a[0] + b[0], a[1])
    if a[1] > 0:
        return (a[0] - b[0], 1)
    return (b[0] - a[0], 1)


def _sub(a, b):
    return _add(a, _neg(b))


def _mul(c, a):
    if a is None or abs(c) < 1e-12:
        return None
    if abs(abs(c) - 1.0) < 1e-12:
        return (a[0], a[1] * (1 if c > 0 else -1))
    return (a[0] * np.float32(c * a[1]), 1)


def _cadd(a, b):
    return (_add(a[0], b[0]), _add(a[1], b[1]))


def _csub(a, b):
    return (_sub(a[0], b[0]), _sub(a[1], b[1]))


def _cscale(c, a):
    return (_mul(c, a[0]), _mul(c, a[1]))


def _dft4(x):
    s0, d0 = _cadd(x[0], x[2]), _csub(x[0], x[2])
    s1, d1 = _cadd(x[1], x[3]), _csub(x[1], x[3])
    x1 = (_add(d0[0], d1[1]), _sub(d0[1], d1[0]))
    x3 = (_sub(d0[0], d1[1]), _add(d0[1], d1[0]))
    return [_cadd(s0, s1), x1, _csub(s0, s1), x3]


_C1 = math.cos(2 * math.pi / 5)
_C2 = math.cos(4 * math.pi / 5)
_S1 = math.sin(2 * math.pi / 5)
_S2 = math.sin(4 * math.pi / 5)


def _dft5(x):
    t1, t3 = _cadd(x[1], x[4]), _csub(x[1], x[4])
    t2, t4 = _cadd(x[2], x[3]), _csub(x[2], x[3])
    t5 = _cadd(t1, t2)
    x0 = _cadd(x[0], t5)
    m2 = _cadd(x[0], _cscale((_C1 + _C2) / 2, t5))
    m3 = _cscale((_C1 - _C2) / 2, _csub(t1, t2))
    s1, s2 = _cadd(m2, m3), _csub(m2, m3)
    u = _cadd(_cscale(_S1, t3), _cscale(_S2, t4))
    v = _csub(_cscale(_S2, t3), _cscale(_S1, t4))
    x1 = (_add(s1[0], u[1]), _sub(s1[1], u[0]))
    x4 = (_sub(s1[0], u[1]), _add(s1[1], u[0]))
    x2 = (_add(s2[0], v[1]), _sub(s2[1], v[0]))
    x3 = (_sub(s2[0], v[1]), _add(s2[1], v[0]))
    return [x0, x1, x2, x3, x4]


def _fft20(load, emit, inverse=False, real_input=False):
    def sw(z):
        return (z[1], z[0]) if inverse else z

    a = [_dft4([sw(load((5 * n1 + 4 * n2) % 20)) for n1 in range(4)]) for n2 in range(5)]
    for k1 in range(4):
        if real_input and k1 == 3:
            continue
        r = _dft5([a[n2][k1] for n2 in range(5)])
        for k2 in range(5):
            k = (5 * k1 + 16 * k2) % 20
            emit(k, sw(r[k2]))
            if real_input and k1 == 1:
                emit(20 - k, (r[k2][0], _neg(r[k2][1])))


def _val(a):
    return a[0] if a[1] > 0 else -a[0]


def _pos(arr):
    return (arr, 1)


def _sym7(x, scale=1.0):
    sm = [_add(x[3 + j], x[3 - j]) for j in (1, 2, 3)]
    df = [_sub(x[3 + j], x[3 - j]) for j in (1, 2, 3)]
    x0 = _mul(scale, x[3])

    def cs(k):
        acc = x0
        for j in (1, 2, 3):
            acc = _add(acc, _mul(scale * math.cos(2 * math.pi * k * j / T), sm[j - 1]))
        return acc

    def sn(k):
        acc = None
        for j in (1, 2, 3):
            acc = _add(acc, _mul(scale * math.sin(2 * math.pi * k * j / T), df[j - 1]))
        return acc

    return cs, sn


NCH = 8
HC = H // NCH
NQ = 4


def _kernel(x_hbm, w_ref, f_ref, g_ref, o_hbm,
            xbuf, wf, wt, what, x2a, x2b, y2a, y2b, isem, osem, *xy):
    obuf = xbuf
    x2 = (x2a, x2b)
    y2 = (y2a, y2b)

    def in_copy(k):
        return pltpu.make_async_copy(
            x_hbm.at[pl.ds(k * HC, HC)], xbuf.at[pl.ds(k * HC, HC)], isem.at[k])

    def out_copy(k):
        return pltpu.make_async_copy(
            obuf.at[pl.ds(k * HC, HC)], o_hbm.at[pl.ds(k * HC, HC)], osem.at[k])

    with jax.named_scope('P0'):
        for k in range(NCH):
            in_copy(k).start()

    with jax.named_scope('P1'):
        wf[...] = w_ref[...].astype(F32)

    def w_pieces(ib):
        rows = pl.ds(pl.multiple_of(ib * 8, 8), 8)

        def stage1(a):
            cs, sn = _sym7([_pos(wf[a * K + b, rows, :]) for b in range(K)], 1.0 / T)
            for v in range(11):
                wt[a, 2 * v if v < 10 else 1] = _val(cs(v))
                if 0 < v < 10:
                    wt[a, 2 * v + 1] = _val(_neg(sn(v)))

        def put(q, wr, wi):
            what[q, rows, :] = _val(wr)
            if wi is not None:
                what[q + 1, rows, :] = _val(_add(wr, wi))
                what[q + 2, rows, :] = _val(_sub(wi, wr))

        def stage2(v):
            rc, rs = _sym7([_pos(wt[a, 2 * v if v < 10 else 1]) for a in range(K)], 1.0 / T)
            if v in (0, 10):
                base = 540 + (0 if v == 0 else 29)
                for u in range(11):
                    if u in (0, 10):
                        put(base + _real_q(u), rc(u), None)
                    else:
                        put(base + _real_q(u), rc(u), _neg(rs(u)))
                return
            ic, is_ = _sym7([_pos(wt[a, 2 * v + 1]) for a in range(K)], 1.0 / T)
            base = 60 * (v - 1)
            for u in range(11):
                a_, b_ = rc(u), ic(u)
                if u in (0, 10):
                    put(base + 3 * u, a_, b_)
                else:
                    c_, d_ = rs(u), is_(u)
                    put(base + 3 * u, _add(a_, d_), _sub(b_, c_))
                    put(base + 3 * (T - u), _sub(a_, d_), _add(b_, c_))

        return ([lambda a=a: stage1(a) for a in range(K)]
                + [lambda v=v: stage2(v) for v in range(11)])

    nt = (((1,), (1,)), ((), ()))

    def s1_row(h):
        xa = xbuf[h, :, pl.ds(0, 128)]
        xb = xbuf[h, :, pl.ds(128, 96)]
        w0 = jnp.concatenate([xa[:, :112], xb[:, 90:96], xa[:, 118:128]], axis=1)
        w1 = jnp.concatenate([xb, xa[:, 96:128]], axis=1)
        r0 = lax.dot_general(f_ref[0], w0, nt, preferred_element_type=F32)
        r1 = lax.dot_general(f_ref[1], w1, nt, preferred_element_type=F32)
        for v in range(10):
            xy[v][h + 6, pl.ds(0, 16), :] = r0[16 * v:16 * v + 16]
            xy[v][h + 6, pl.ds(16, 16), :] = r1[16 * v:16 * v + 16]

    def a_body(k, carry):
        wp = []
        for i in range(3):
            wp += w_pieces(3 * k + i)
        for j in range(2 * HC):
            if j % HC == 0:
                in_copy(2 * k + j // HC).wait()
            s1_row(2 * HC * k + j)
            for f in wp[j * len(wp) // (2 * HC):(j + 1) * len(wp) // (2 * HC)]:
                f()
        return carry

    with jax.named_scope('A'):
        lax.fori_loop(0, NCH // 2, a_body, 0)
    with jax.named_scope('P2'):
        for v in range(10):
            xy[v][pl.ds(0, 6)] = xy[v][pl.ds(H, 6)]

    def ld1(slot, g, v, part):
        return xy[v][slot, pl.ds(g * 16 + part, 8, stride=2), :]

    def st1(slot, g, v, part, val):
        xy[v][slot, pl.ds(g * 16 + part, 8, stride=2), :] = val

    def s2_one(kind, v, par, th, g):
        row = pl.ds(pl.multiple_of(th * 16 + g * 8, 8), 8)

        def put(q, z):
            if z[1] is None:
                x2[par][q, row, :] = _val(z[0])
            else:
                x2[par][q, row, :] = _val(_add(z[0], z[1]))
                x2[par][q + 1, row, :] = _val(z[1])
                x2[par][q + 2, row, :] = _val(z[0])

        if kind == "c":
            _fft20(lambda a: (_pos(ld1(V * th + a, g, v, 0)), _pos(ld1(V * th + a, g, v, 1))),
                   lambda u, z: put(3 * u, z))
        else:
            for vi in range(2):
                def emit(u, z, vi=vi):
                    if u <= 10:
                        put(29 * vi + _real_q(u), (z[0], None) if u in (0, 10) else z)
                _fft20(lambda a, vi=vi: (_pos(ld1(V * th + a, g, 0, vi)), None), emit,
                       real_input=True)

    def s3_plane(par, q, wq):
        y2[par][q] = jnp.dot(x2[par][q], what[wq], preferred_element_type=F32)

    def s3_piece(kind, v, par, t):
        if kind == "c":
            return [lambda i=i: s3_plane(par, 15 * t + i, 60 * (v - 1) + 15 * t + i)
                    for i in range(15)]
        return [lambda q=q: s3_plane(par, q, 540 + q) for q in range(58)[t::NQ]]

    def yval(par, q, row, real):
        k1 = y2[par][q, row, :]
        if real:
            return (_pos(k1), None)
        return (_pos(k1 - y2[par][q + 1, row, :]), _pos(k1 + y2[par][q + 2, row, :]))

    def s4_one(kind, v, par, th, g):
        row = pl.ds(pl.multiple_of(th * 16 + g * 8, 8), 8)
        if kind == "c":
            def emit(a, z):
                if SH <= a < SH + V:
                    st1(V * th + a - SH + 6, g, v, 0, _val(z[0]))
                    st1(V * th + a - SH + 6, g, v, 1, _val(z[1]))
            _fft20(lambda u: yval(par, 3 * u, row, False), emit, inverse=True)
        else:
            for vi in range(2):
                cache = {}

                def load(u, vi=vi, cache=cache):
                    uu = u if u <= 10 else T - u
                    if uu not in cache:
                        cache[uu] = yval(par, 29 * vi + _real_q(uu), row, uu in (0, 10))
                    re, im = cache[uu]
                    return (re, im) if u <= 10 else (re, _neg(im))

                def emit(a, z, vi=vi):
                    if SH <= a < SH + V:
                        st1(V * th + a - SH + 6, g, 0, vi, _val(z[0]))
                _fft20(load, emit, inverse=True)

    def slot(s2, s3, s4):
        def piece(t):
            mm = s3_piece(s3[0], s3[1], s3[2], t) if s3 else []
            n = 2 * NT // NQ
            for i in range(n):
                th, g = t * (NT // NQ) + i // 2, i % 2
                for f in mm[2 * i:2 * i + 1]:
                    f()
                if s2:
                    s2_one(s2[0], s2[1], s2[2], th, g)
                for f in mm[2 * i + 1:2 * i + 2]:
                    f()
                if s4:
                    s4_one(s4[0], s4[1], s4[2], th, g)

        if s3 and s3[0] == "r":
            for t in range(NQ):
                piece(t)
        else:
            def body(t, carry):
                piece(t)
                return carry
            lax.fori_loop(0, NQ, body, 0)

    with jax.named_scope('B0'):
        slot(("c", 1, 0), None, None)
    with jax.named_scope('B1'):
        slot(("c", 2, 1), ("c", 1, 0), None)
    with jax.named_scope('Bmain'):
        for v in range(3, 10):
            par = v % 2
            slot(("c", v, 1 - par), ("c", v - 1, par), ("c", v - 2, 1 - par))
    with jax.named_scope('B9'):
        slot(("r", 0, 1), ("c", 9, 0), ("c", 8, 1))
    with jax.named_scope('B10'):
        slot(None, ("r", 0, 1), ("c", 9, 0))
    with jax.named_scope('B11'):
        slot(None, None, ("r", 0, 1))

    def s5_body(k, carry):
        for j in range(HC):
            h = k * HC + j
            parts = [jnp.dot(g_ref[...],
                             jnp.concatenate([xy[v][h + 6, pl.ds(8 * jj, 8), :]
                                              for v in range(10)], axis=0),
                             preferred_element_type=F32) for jj in range(4)]
            y = jnp.concatenate(parts, axis=0)
            obuf[h] = y.T.astype(BF16)
        out_copy(k).start()
        return carry

    with jax.named_scope('C'):
        lax.fori_loop(0, NCH, s5_body, 0)
    with jax.named_scope('E'):
        for k in range(NCH):
            out_copy(k).wait()


@jax.jit
def pallas_standalone__fft_conv__vision_kernel(x: jax.Array, w: jax.Array):
    assert x.shape == (1, H, W, C) and w.shape == (K, K, C, C)
    xt = jnp.transpose(x.reshape(H, W, C), (0, 2, 1))
    w2 = w.reshape(K * K, C, C)
    vmem = pl.BlockSpec(memory_space=pltpu.VMEM)
    out = pl.pallas_call(
        _kernel,
        out_shape=jax.ShapeDtypeStruct((H, C, W), BF16),
        in_specs=[pl.BlockSpec(memory_space=pl.ANY), vmem, vmem, vmem],
        out_specs=pl.BlockSpec(memory_space=pl.ANY),
        scratch_shapes=[
            pltpu.VMEM((H, C, W), BF16),
            pltpu.VMEM((K * K, C, C), F32),
            pltpu.VMEM((K, T, 8, C), F32),
            pltpu.VMEM((NPL, C, C), F32),
            pltpu.VMEM((60, 256, C), F32),
            pltpu.VMEM((60, 256, C), F32),
            pltpu.VMEM((60, 256, C), F32),
            pltpu.VMEM((60, 256, C), F32),
            pltpu.SemaphoreType.DMA((NCH,)),
            pltpu.SemaphoreType.DMA((NCH,)),
        ] + [pltpu.VMEM((NSLOT, 32, C), F32) for _ in range(10)],
        compiler_params=pltpu.CompilerParams(vmem_limit_bytes=127 * 1024 * 1024, flags=_FLAGS),
        name="fft_conv_vision",
    )(xt, w2, _F.astype(BF16), _G)
    return jnp.transpose(out, (0, 2, 1)).reshape(1, H, W, C)
```

```python
import math

import numpy as np
import jax
import jax.numpy as jnp
from jax import lax
import jax.experimental.pallas as pl
import jax.experimental.pallas.tpu as pltpu

H = 224
W = 224
C = 96
K = 7
T = 20
V = 14
NT = 8
HB = H // 2
SB = HB + 6
NSLOT = 2 * SB
NPL = 598
SH = 3

_FLAGS = {}
F32 = jnp.float32
BF16 = jnp.bfloat16


def _plane_fwd(p, b):
    if p == 0:
        return 1.0
    if p == T - 1:
        return -1.0 if b % 2 else 1.0
    v = (p + 1) // 2
    ang = 2.0 * math.pi * v * b / T
    return math.cos(ang) if p % 2 == 1 else -math.sin(ang)


def _plane_inv(p, b):
    if p == 0:
        return 1.0
    if p == T - 1:
        return -1.0 if b % 2 else 1.0
    v = (p + 1) // 2
    ang = 2.0 * math.pi * v * b / T
    return 2.0 * math.cos(ang) if p % 2 == 1 else -2.0 * math.sin(ang)


def _vp(v, pl_):
    if v == 0:
        return 0 if pl_ == 0 else T - 1
    return 2 * v - 1 + pl_


def _make_f():
    f = np.zeros((2, 8 * T, 128), np.float32)
    for g in range(2):
        for tl in range(8):
            for b in range(T):
                w = V * (8 * g + tl) - 6 + b
                if g == 0:
                    lane = w if w >= 0 else 112 + (w + 6)
                else:
                    lane = w if w < 128 else w - 128
                for v in range(10):
                    for pl_ in range(2):
                        f[g, v * 16 + tl * 2 + pl_, lane] = _plane_fwd(_vp(v, pl_), b)
    return f


def _make_g():
    g = np.zeros((4 * V, 4 * T), np.float32)
    for tl in range(4):
        for b in range(V):
            for v in range(10):
                for pl_ in range(2):
                    g[tl * V + b, v * 8 + tl * 2 + pl_] = _plane_inv(_vp(v, pl_), b + SH)
    return g


_F = _make_f()
_G = _make_g()


def _real_q(u):
    return 0 if u == 0 else (28 if u == 10 else 1 + 3 * (u - 1))


def _neg(a):
    return None if a is None else (a[0], -a[1])


def _add(a, b):
    if a is None:
        return b
    if b is None:
        return a
    if a[1] == b[1]:
        return (a[0] + b[0], a[1])
    if a[1] > 0:
        return (a[0] - b[0], 1)
    return (b[0] - a[0], 1)


def _sub(a, b):
    return _add(a, _neg(b))


def _mul(c, a):
    if a is None or abs(c) < 1e-12:
        return None
    if abs(abs(c) - 1.0) < 1e-12:
        return (a[0], a[1] * (1 if c > 0 else -1))
    return (a[0] * np.float32(c * a[1]), 1)


def _cadd(a, b):
    return (_add(a[0], b[0]), _add(a[1], b[1]))


def _csub(a, b):
    return (_sub(a[0], b[0]), _sub(a[1], b[1]))


def _cscale(c, a):
    return (_mul(c, a[0]), _mul(c, a[1]))


def _dft4(x):
    s0, d0 = _cadd(x[0], x[2]), _csub(x[0], x[2])
    s1, d1 = _cadd(x[1], x[3]), _csub(x[1], x[3])
    x1 = (_add(d0[0], d1[1]), _sub(d0[1], d1[0]))
    x3 = (_sub(d0[0], d1[1]), _add(d0[1], d1[0]))
    return [_cadd(s0, s1), x1, _csub(s0, s1), x3]


_C1 = math.cos(2 * math.pi / 5)
_C2 = math.cos(4 * math.pi / 5)
_S1 = math.sin(2 * math.pi / 5)
_S2 = math.sin(4 * math.pi / 5)


def _dft5(x):
    t1, t3 = _cadd(x[1], x[4]), _csub(x[1], x[4])
    t2, t4 = _cadd(x[2], x[3]), _csub(x[2], x[3])
    t5 = _cadd(t1, t2)
    x0 = _cadd(x[0], t5)
    m2 = _cadd(x[0], _cscale((_C1 + _C2) / 2, t5))
    m3 = _cscale((_C1 - _C2) / 2, _csub(t1, t2))
    s1, s2 = _cadd(m2, m3), _csub(m2, m3)
    u = _cadd(_cscale(_S1, t3), _cscale(_S2, t4))
    v = _csub(_cscale(_S2, t3), _cscale(_S1, t4))
    x1 = (_add(s1[0], u[1]), _sub(s1[1], u[0]))
    x4 = (_sub(s1[0], u[1]), _add(s1[1], u[0]))
    x2 = (_add(s2[0], v[1]), _sub(s2[1], v[0]))
    x3 = (_sub(s2[0], v[1]), _add(s2[1], v[0]))
    return [x0, x1, x2, x3, x4]


def _fft20(load, emit, inverse=False, real_input=False):
    def sw(z):
        return (z[1], z[0]) if inverse else z

    a = [_dft4([sw(load((5 * n1 + 4 * n2) % 20)) for n1 in range(4)]) for n2 in range(5)]
    for k1 in range(4):
        if real_input and k1 == 3:
            continue
        r = _dft5([a[n2][k1] for n2 in range(5)])
        for k2 in range(5):
            k = (5 * k1 + 16 * k2) % 20
            emit(k, sw(r[k2]))
            if real_input and k1 == 1:
                emit(20 - k, (r[k2][0], _neg(r[k2][1])))


def _val(a):
    return a[0] if a[1] > 0 else -a[0]


def _pos(arr):
    return (arr, 1)


def _sym7(x, scale=1.0):
    sm = [_add(x[3 + j], x[3 - j]) for j in (1, 2, 3)]
    df = [_sub(x[3 + j], x[3 - j]) for j in (1, 2, 3)]
    x0 = _mul(scale, x[3])

    def cs(k):
        acc = x0
        for j in (1, 2, 3):
            acc = _add(acc, _mul(scale * math.cos(2 * math.pi * k * j / T), sm[j - 1]))
        return acc

    def sn(k):
        acc = None
        for j in (1, 2, 3):
            acc = _add(acc, _mul(scale * math.sin(2 * math.pi * k * j / T), df[j - 1]))
        return acc

    return cs, sn


NCH = 8
HC = H // NCH
NQ = 2


def _kernel(x_hbm, w_ref, f_ref, g_ref, o_hbm,
            xbuf, obuf, wf, wt, what, x2a, x2b, y2a, y2b, isem, osem, *xy):
    x2 = (x2a, x2b)
    y2 = (y2a, y2b)

    def in_copy(k):
        return pltpu.make_async_copy(
            x_hbm.at[pl.ds(k * HC, HC)], xbuf.at[pl.ds(k * HC, HC)], isem.at[k])

    def out_copy(k):
        return pltpu.make_async_copy(
            obuf.at[pl.ds(k * HC, HC)], o_hbm.at[pl.ds(k * HC, HC)], osem.at[k])

    for k in (NCH - 1,) + tuple(range(NCH - 1)):
        in_copy(k).start()

    wf[...] = w_ref[...].astype(F32)

    def w_pieces(ib):
        rows = pl.ds(ib * 8, 8)

        def stage1(a):
            cs, sn = _sym7([_pos(wf[a * K + b, rows, :]) for b in range(K)], 1.0 / T)
            for v in range(11):
                wt[a, 2 * v if v < 10 else 1] = _val(cs(v))
                if 0 < v < 10:
                    wt[a, 2 * v + 1] = _val(_neg(sn(v)))

        def put(q, wr, wi):
            what[q, rows, :] = _val(wr)
            if wi is not None:
                what[q + 1, rows, :] = _val(_add(wr, wi))
                what[q + 2, rows, :] = _val(_sub(wi, wr))

        def stage2(v):
            rc, rs = _sym7([_pos(wt[a, 2 * v if v < 10 else 1]) for a in range(K)], 1.0 / T)
            if v in (0, 10):
                base = 540 + (0 if v == 0 else 29)
                for u in range(11):
                    if u in (0, 10):
                        put(base + _real_q(u), rc(u), None)
                    else:
                        put(base + _real_q(u), rc(u), _neg(rs(u)))
                return
            ic, is_ = _sym7([_pos(wt[a, 2 * v + 1]) for a in range(K)], 1.0 / T)
            base = 60 * (v - 1)
            for u in range(11):
                a_, b_ = rc(u), ic(u)
                if u in (0, 10):
                    put(base + 3 * u, a_, b_)
                else:
                    c_, d_ = rs(u), is_(u)
                    put(base + 3 * u, _add(a_, d_), _sub(b_, c_))
                    put(base + 3 * (T - u), _sub(a_, d_), _add(b_, c_))

        return ([lambda a=a: stage1(a) for a in range(K)]
                + [lambda v=v: stage2(v) for v in range(11)])

    nt = (((1,), (1,)), ((), ()))

    def s1_row(h, slot):
        xa = xbuf[h, :, pl.ds(0, 128)]
        xb = xbuf[h, :, pl.ds(128, 96)]
        w0 = jnp.concatenate([xa[:, :112], xb[:, 90:96], xa[:, 118:128]], axis=1)
        w1 = jnp.concatenate([xb, xa[:, 96:128]], axis=1)
        r0 = lax.dot_general(f_ref[0], w0, nt, preferred_element_type=F32)
        r1 = lax.dot_general(f_ref[1], w1, nt, preferred_element_type=F32)
        for v in range(10):
            xy[v][slot, pl.ds(0, 16), :] = r0[16 * v:16 * v + 16]
            xy[v][slot, pl.ds(16, 16), :] = r1[16 * v:16 * v + 16]

    wp = []
    for ib in range(C // 8):
        wp += w_pieces(ib)
    in_copy(NCH - 1).wait()
    for j in range(SB):
        if j >= 6 and (j - 6) % HC == 0:
            in_copy((j - 6) // HC).wait()
        s1_row((j - 6) % H, j)
        for f in wp[j * len(wp) // SB:(j + 1) * len(wp) // SB]:
            f()

    def s1_second_half():
        for k in range(NCH // 2, NCH - 1):
            in_copy(k).wait()

        def body(k, carry):
            for j in range(HC):
                s1_row(HB + k * HC + j, SB + 6 + k * HC + j)
            return carry
        lax.fori_loop(0, NCH // 2, body, 0)
        for j in range(6):
            s1_row(HB - 6 + j, SB + j)

    def ld1(slot, g, v, part):
        return xy[v][slot, pl.ds(g * 16 + part, 8, stride=2), :]

    def st1(slot, g, v, part, val):
        xy[v][slot, pl.ds(g * 16 + part, 8, stride=2), :] = val

    def s2_one(kind, v, par, th, g):
        row = pl.ds(th[0] + (th[2] * 16 + g * 8), 8)

        def put(q, z):
            if z[1] is None:
                x2[par][q, row, :] = _val(z[0])
            else:
                x2[par][q, row, :] = _val(_add(z[0], z[1]))
                x2[par][q + 1, row, :] = _val(z[1])
                x2[par][q + 2, row, :] = _val(z[0])

        if kind == "c":
            _fft20(lambda a: (_pos(ld1(th[1] + (V * th[2] + a), g, v, 0)), _pos(ld1(th[1] + (V * th[2] + a), g, v, 1))),
                   lambda u, z: put(3 * u, z))
        else:
            for vi in range(2):
                def emit(u, z, vi=vi):
                    if u <= 10:
                        put(29 * vi + _real_q(u), (z[0], None) if u in (0, 10) else z)
                _fft20(lambda a, vi=vi: (_pos(ld1(th[1] + (V * th[2] + a), g, 0, vi)), None), emit,
                       real_input=True)

    def s3_plane(par, q, wq):
        y2[par][q] = jnp.dot(x2[par][q], what[wq], preferred_element_type=F32)

    def s3_piece(kind, v, par, t):
        if kind == "c":
            n = 60 // NQ
            nt_ = n * t
            return [lambda i=i: s3_plane(par, nt_ + i, nt_ + (60 * (v - 1) + i))
                    for i in range(n)]
        return [lambda q=q: s3_plane(par, q, 540 + q) for q in range(58)[t::NQ]]

    def yval(par, q, row, real):
        k1 = y2[par][q, row, :]
        if real:
            return (_pos(k1), None)
        return (_pos(k1 - y2[par][q + 1, row, :]), _pos(k1 + y2[par][q + 2, row, :]))

    def s4_one(kind, v, par, th, g):
        row = pl.ds(th[0] + (th[2] * 16 + g * 8), 8)
        if kind == "c":
            def emit(a, z):
                if SH <= a < SH + V:
                    st1(th[1] + (V * th[2] + a - SH + 6), g, v, 0, _val(z[0]))
                    st1(th[1] + (V * th[2] + a - SH + 6), g, v, 1, _val(z[1]))
            _fft20(lambda u: yval(par, 3 * u, row, False), emit, inverse=True)
        else:
            for vi in range(2):
                cache = {}

                def load(u, vi=vi, cache=cache):
                    uu = u if u <= 10 else T - u
                    if uu not in cache:
                        cache[uu] = yval(par, 29 * vi + _real_q(uu), row, uu in (0, 10))
                    re, im = cache[uu]
                    return (re, im) if u <= 10 else (re, _neg(im))

                def emit(a, z, vi=vi):
                    if SH <= a < SH + V:
                        st1(th[1] + (V * th[2] + a - SH + 6), g, 0, vi, _val(z[0]))
                _fft20(load, emit, inverse=True)

    half = [0]

    def slot(s2, s3, s4):
        def piece(t):
            mm = s3_piece(s3[0], s3[1], s3[2], t) if s3 else []
            n = 2 * NT // NQ
            rb = pl.multiple_of(t * (16 * NT // NQ), 8)
            sb = half[0] * SB + t * (V * NT // NQ)
            for i in range(n):
                th, g = (rb, sb, i // 2), i % 2
                for f in mm[2 * i * len(mm) // (2 * n):(2 * i + 1) * len(mm) // (2 * n)]:
                    f()
                if s2:
                    s2_one(s2[0], s2[1], s2[2], th, g)
                for f in mm[(2 * i + 1) * len(mm) // (2 * n):(2 * i + 2) * len(mm) // (2 * n)]:
                    f()
                if s4:
                    s4_one(s4[0], s4[1], s4[2], th, g)

        if s3 and s3[0] == "r":
            for t in range(NQ):
                piece(t)
        else:
            def body(t, carry):
                piece(t)
                return carry
            lax.fori_loop(0, NQ, body, 0)

    def s5_chunk(k, slot0):
        for j in range(HC):
            parts = [jnp.dot(g_ref[...],
                             jnp.concatenate([xy[v][slot0 + j, pl.ds(8 * jj, 8), :]
                                              for v in range(10)], axis=0),
                             preferred_element_type=F32) for jj in range(4)]
            y = jnp.concatenate(parts, axis=0)
            obuf[k * HC + j] = y.T.astype(BF16)
        out_copy(k).start()

    def half_body(b, carry):
        half[0] = b

        @pl.when(b == 1)
        def _():
            s1_second_half()

        slot(("c", 1, 0), None, None)
        slot(("c", 2, 1), ("c", 1, 0), None)
        for v in range(3, 10):
            par = v % 2
            slot(("c", v, 1 - par), ("c", v - 1, par), ("c", v - 2, 1 - par))
        slot(("r", 0, 1), ("c", 9, 0), ("c", 8, 1))
        slot(None, ("r", 0, 1), ("c", 9, 0))
        slot(None, None, ("r", 0, 1))

        def s5_body(k, c2):
            s5_chunk(b * (NCH // 2) + k, b * SB + 6 + k * HC)
            return c2
        lax.fori_loop(0, NCH // 2, s5_body, 0)
        return carry

    lax.fori_loop(0, 2, half_body, 0)
    for k in range(NCH):
        out_copy(k).wait()


@jax.jit
def pallas_standalone__fft_conv__vision_kernel(x: jax.Array, w: jax.Array):
    assert x.shape == (1, H, W, C) and w.shape == (K, K, C, C)
    xt = jnp.transpose(x.reshape(H, W, C), (0, 2, 1))
    w2 = w.reshape(K * K, C, C)
    vmem = pl.BlockSpec(memory_space=pltpu.VMEM)
    out = pl.pallas_call(
        _kernel,
        out_shape=jax.ShapeDtypeStruct((H, C, W), BF16),
        in_specs=[pl.BlockSpec(memory_space=pl.ANY), vmem, vmem, vmem],
        out_specs=pl.BlockSpec(memory_space=pl.ANY),
        scratch_shapes=[
            pltpu.VMEM((H, C, W), BF16),
            pltpu.VMEM((H, C, W), BF16),
            pltpu.VMEM((K * K, C, C), F32),
            pltpu.VMEM((K, T, 8, C), F32),
            pltpu.VMEM((NPL, C, C), F32),
            pltpu.VMEM((60, 16 * NT, C), F32),
            pltpu.VMEM((60, 16 * NT, C), F32),
            pltpu.VMEM((60, 16 * NT, C), F32),
            pltpu.VMEM((60, 16 * NT, C), F32),
            pltpu.SemaphoreType.DMA((NCH,)),
            pltpu.SemaphoreType.DMA((NCH,)),
        ] + [pltpu.VMEM((NSLOT, 32, C), F32) for _ in range(10)],
        compiler_params=pltpu.CompilerParams(vmem_limit_bytes=127 * 1024 * 1024, flags=_FLAGS),
        name="fft_conv_vision",
    )(xt, w2, _F.astype(BF16), _G)
    return jnp.transpose(out, (0, 2, 1)).reshape(1, H, W, C)
```
